```python
import jax
import jax.numpy as jnp

def _softmax(x, axis=-1):
    return jax.nn.softmax(x, axis=axis)
def _gelu(x):
    return jax.nn.gelu(x, approximate=True)
def _silu(x):
    return jax.nn.silu(x)
def _sigmoid(x):
    return jax.nn.sigmoid(x)
def _layernorm(x, axis=-1, eps=1e-5):
    m = jnp.mean(x, axis=axis, keepdims=True)
    v = jnp.var(x, axis=axis, keepdims=True)
    return (x - m) / jnp.sqrt(v + eps)
def _scatter_add(tgt, idx, src, axis=0):
    return tgt.at[idx].add(src)
def _segment_sum(src, seg, n):
    return jax.ops.segment_sum(src, seg, n)
class _Rng:
    def __init__(self, key):
        self._k = key
    def _next(self):
        self._k, sub = jax.random.split(self._k)
        return sub
    def normal(self, shape):
        return jax.random.normal(self._next(), shape, dtype=jnp.bfloat16)
    def randint(self, lo, hi, shape):
        return jax.random.randint(self._next(), shape, lo, hi, dtype=jnp.int32)
    def uniform(self, shape, lo=0.0, hi=1.0):
        return jax.random.uniform(self._next(), shape, jnp.bfloat16, lo, hi)
    def permutation(self, n):
        return jax.random.permutation(self._next(), n)


kernel_name = 'standalone__instancenorm__prompt'

def setup_inputs():
    _rng = _Rng(jax.random.key(int.from_bytes(__import__("os").urandom(4), "little")))
    _w = (lambda a: (lambda t: t.astype(jnp.bfloat16) if jnp.issubdtype(t.dtype, jnp.floating) else t)(jnp.asarray(a)))
    B, C, H, W = 2, 1024, 2048, 32
    return {
        "x": _w((lambda *s: _rng.normal(s) * 0.05)(B, C, H, W)),
        "g": _w((lambda *s: _rng.normal(s) * 0.05)(C) + 1.0),
        "b": _w((lambda *s: _rng.normal(s) * 0.05)(C)),
    }

def reference(x, g, b):
    mu = x.mean(axis=(-2, -1), keepdims=True)
    var = ((x - mu) * (x - mu)).mean(axis=(-2, -1), keepdims=True)
    xhat = (x - mu) / jnp.sqrt(var + 1e-5)
    return xhat * g.reshape(1, -1, 1, 1) + b.reshape(1, -1, 1, 1)
```

```python
import functools
import jax, jax.numpy as jnp
from jax import lax
from jax.experimental import pallas as pl
from jax.experimental.pallas import tpu as pltpu

def make(S=8, K=64, D=2, rq=2, wq=4, rpr=2, wpr=2, compute=True, wcols=1):
    def kernel(x_hbm, g_ref, b_ref, o_hbm, buf, rsem, wsem):
        _, P, W, H = x_hbm.shape
        C = g_ref.shape[0]*128
        nchunk = P//K
        inv_n = 1.0/(W*H)
        def rd_start(c, k):
            for q in range(rq):
                r = W//rq
                for j in range(S):
                    pltpu.make_async_copy(x_hbm.at[j, c*K+k, pl.ds(q*r,r)], buf.at[k, j, pl.ds(q*r,r)], rsem.at[k]).start(priority=j%rpr)
        def rd_wait(k):
            pltpu.make_async_copy(buf.at[k], buf.at[k], rsem.at[k]).wait()
        def wr_start(c, k):
            for q in range(wq):
                r = W//wq
                for h in range(wcols):
                    cc = H//wcols
                    for j in range(S):
                        pltpu.make_async_copy(buf.at[k, j, pl.ds(q*r,r), pl.ds(h*cc,cc)], o_hbm.at[j, c*K+k, pl.ds(q*r,r), pl.ds(h*cc,cc)], wsem.at[k]).start(priority=j%wpr)
        def wr_wait(k):
            pltpu.make_async_copy(buf.at[k], buf.at[k], wsem.at[k]).wait()

        gv = g_ref[...].astype(jnp.float32); bv = b_ref[...].astype(jnp.float32)
        lane = lax.broadcasted_iota(jnp.int32, gv.shape, 1)

        def norm_slot(c, k):
            i = c*K + k
            m = lane == (i % 128)
            gs = jnp.sum(jnp.where(m, gv, 0.0), axis=1, keepdims=True)
            bs = jnp.sum(jnp.where(m, bv, 0.0), axis=1, keepdims=True)
            rows_per = P//128
            ii = i//128
            def pick(t, j):
                r0 = ((j*P) % C)//128
                out = t[r0:r0+1]
                for u in range(1, rows_per):
                    out = jnp.where(ii == u, t[r0+u:r0+u+1], out)
                return out
            TW = 256
            def tiles(j):
                for r in range(0, W, 16):
                    for h in range(0, H, TW):
                        yield r, h
            def red(acc):
                s = jnp.sum(acc, axis=0, keepdims=True)
                return jnp.sum(s, axis=1, keepdims=True)
            def fold(v):
                v = v[:8] + v[8:]
                a = v[:, :128]
                for h in range(128, TW, 128): a = a + v[:, h:h+128]
                return a
            mus = []
            for j in range(S):
                acc = None
                for r,h in tiles(j):
                    v = buf[k, j, pl.ds(r,16), pl.ds(h,TW)].astype(jnp.float32)
                    acc = v if acc is None else acc + v
                mus.append(red(fold(acc))*inv_n)
            sc=[]; sh=[]
            for j in range(S):
                acc = None
                for r,h in tiles(j):
                    v = buf[k, j, pl.ds(r,16), pl.ds(h,TW)].astype(jnp.float32) - mus[j]
                    acc = v*v if acc is None else acc + v*v
                var = red(fold(acc))*inv_n
                a = pick(gs, j)*lax.rsqrt(var + 1e-5)
                sc.append(a); sh.append(pick(bs, j) - mus[j]*a)
            for j in range(S):
                for r,h in tiles(j):
                    v = buf[k, j, pl.ds(r,16), pl.ds(h,TW)].astype(jnp.float32)
                    buf[k, j, pl.ds(r,16), pl.ds(h,TW)] = (v*sc[j] + sh[j]).astype(buf.dtype)

        for k in range(D): rd_start(0, k)
        def chunk(c, _):
            def rbody(k, _):
                rd_wait(k)
                @pl.when(k + D < K)
                def _(): rd_start(c, k + D)
                @pl.when(k + D >= K)
                def _(): wr_start(c, k + D - K)
                if compute: norm_slot(c, k)
            lax.fori_loop(0, K, rbody, None)
            def wbody(k, _):
                wr_wait(k)
                @pl.when(k + D < K)
                def _(): wr_start(c, k + D)
                @pl.when(jnp.logical_and(k + D >= K, c + 1 < nchunk))
                def _(): rd_start(c + 1, k + D - K)
            lax.fori_loop(0, K, wbody, None)
        lax.fori_loop(0, nchunk, chunk, None)

    def f(x, g, b):
        B, C, H, W = x.shape
        xt = x.transpose(0,1,3,2).reshape(S, B*C//S, W, H)
        o = pl.pallas_call(kernel,
            in_specs=[pl.BlockSpec(memory_space=pl.ANY), pl.BlockSpec(memory_space=pltpu.VMEM), pl.BlockSpec(memory_space=pltpu.VMEM)],
            out_specs=pl.BlockSpec(memory_space=pl.ANY),
            out_shape=jax.ShapeDtypeStruct(xt.shape, xt.dtype),
            scratch_shapes=[pltpu.VMEM((K,S,W,H), x.dtype), pltpu.SemaphoreType.DMA((K,)), pltpu.SemaphoreType.DMA((K,))],
            compiler_params=pltpu.CompilerParams(vmem_limit_bytes=120*2**20),
        )(xt, g.reshape(C//128,128), b.reshape(C//128,128))
        return o.reshape(B,C,W,H).transpose(0,1,3,2)
    return f


@jax.jit
def pallas_standalone__instancenorm__prompt_kernel(x: jax.Array, g: jax.Array, b: jax.Array):
    return make(D=4)(x, g, b)
```

```python
import jax
import jax.numpy as jnp
from jax import lax
import jax.experimental.pallas as pl
import jax.experimental.pallas.tpu as pltpu

S = 8
K = 86
D = 3
E = 1
NS = 16
RQ, RC = 4, 2
WQ = 4
TW = 256
EPS = 1e-5


def _kernel(x_hbm, g_ref, b_ref, o_hbm, buf, st, rsem, wsem):
    _, P, W, H = x_hbm.shape
    C = g_ref.shape[0] * 128
    nchunk = -(-P // K)
    inv_n = 1.0 / (W * H)

    def rd_start(c, k):
        r, cc = W // RQ, H // RC
        for q in range(RQ):
            for h in range(RC):
                for j in range(S):
                    sl = (pl.ds(q * r, r), pl.ds(h * cc, cc))
                    pltpu.make_async_copy(
                        x_hbm.at[(j, c * K + k) + sl], buf.at[(k, j) + sl], rsem.at[k % NS]
                    ).start(priority=j % 2)

    def wr_start(c, k):
        r = W // WQ
        for q in range(WQ):
            for j in range(S):
                pltpu.make_async_copy(
                    buf.at[k, j, pl.ds(q * r, r)], o_hbm.at[j, c * K + k, pl.ds(q * r, r)],
                    wsem.at[k % NS]
                ).start(priority=j % 2)

    def wait_slot(sem, k):
        pltpu.make_async_copy(buf.at[k], buf.at[k], sem.at[k % NS]).wait()

    gv = g_ref[...].astype(jnp.float32)
    bv = b_ref[...].astype(jnp.float32)
    lane = lax.broadcasted_iota(jnp.int32, gv.shape, 1)

    def norm_slot(c, k):
        i = c * K + k
        m = lane == (i % 128)
        gs = jnp.sum(jnp.where(m, gv, 0.0), axis=1, keepdims=True)
        bs = jnp.sum(jnp.where(m, bv, 0.0), axis=1, keepdims=True)

        def pick(t, j):
            r0 = ((j * P) % C) // 128
            out = t[r0:r0 + 1]
            for u in range(1, P // 128):
                out = jnp.where(i // 128 == u, t[r0 + u:r0 + u + 1], out)
            return out

        tiles = [(r, h) for r in range(0, W, 16) for h in range(0, H, TW)]

        def total(v):
            v = v[:8] + v[8:]
            a = v[:, :128]
            for h in range(128, TW, 128):
                a = a + v[:, h:h + 128]
            return jnp.sum(jnp.sum(a, axis=0, keepdims=True), axis=1, keepdims=True)

        mus = []
        for j in range(S):
            acc = None
            for r, h in tiles:
                v = buf[k, j, pl.ds(r, 16), pl.ds(h, TW)].astype(jnp.float32)
                acc = v if acc is None else acc + v
            mus.append(total(acc) * inv_n)
        kb = jnp.minimum(k, K - 1)
        for j in range(S):
            acc = None
            for r, h in tiles:
                v = buf[kb, j, pl.ds(r, 16), pl.ds(h, TW)].astype(jnp.float32) - mus[j]
                acc = v * v if acc is None else acc + v * v
            a = pick(gs, j) * lax.rsqrt(total(acc) * inv_n + EPS)
            st[0, j] = jnp.broadcast_to(a, (8, 128))
            st[1, j] = jnp.broadcast_to(mus[j], (8, 128))
            st[2, j] = jnp.broadcast_to(pick(bs, j), (8, 128))

        def apply(j, _):
            a = st[0, j]
            s = st[2, j] - st[1, j] * a
            for r in range(0, W, 8):
                for h in range(0, H, 256):
                    v = buf[k, j, pl.ds(r, 8), pl.ds(h, 256)].astype(jnp.float32)
                    o = jnp.concatenate([v[:, :128] * a + s, v[:, 128:] * a + s], axis=1)
                    buf[k, j, pl.ds(r, 8), pl.ds(h, 256)] = o.astype(buf.dtype)
        lax.fori_loop(0, S, apply, None)

    for k in range(D):
        rd_start(0, k)

    def chunk(c, _):
        n = jnp.minimum(K, P - c * K)
        more = c + 1 < nchunk

        def rbody(k, _):
            wait_slot(rsem, k)

            @pl.when(k + D < n)
            def _():
                rd_start(c, k + D)

            @pl.when(k == n - 1 - E)
            def _():
                for u in range(D - E):
                    wr_start(c, u)

            @pl.when(k > n - 1 - E)
            def _():
                wr_start(c, k - n + D)

            norm_slot(c, k)
        lax.fori_loop(0, n, rbody, None)

        def wbody(k, _):
            wait_slot(wsem, k)

            @pl.when(k + D < n)
            def _():
                wr_start(c, k + D)

            @pl.when(jnp.logical_and(k == n - 1 - E, more))
            def _():
                for u in range(D - E):
                    rd_start(c + 1, u)

            @pl.when(jnp.logical_and(k > n - 1 - E, more))
            def _():
                rd_start(c + 1, k - n + D)
        lax.fori_loop(0, n, wbody, None)

    lax.fori_loop(0, nchunk, chunk, None)


@jax.jit
def pallas_standalone__instancenorm__prompt_kernel(x: jax.Array, g: jax.Array, b: jax.Array):
    B, C, H, W = x.shape
    P = B * C // S
    assert P % 128 == 0 and C % P == 0 and W % 32 == 0 and H % 256 == 0
    xt = x.transpose(0, 1, 3, 2).reshape(S, P, W, H)
    o = pl.pallas_call(
        _kernel,
        in_specs=[pl.BlockSpec(memory_space=pl.ANY),
                  pl.BlockSpec(memory_space=pltpu.VMEM),
                  pl.BlockSpec(memory_space=pltpu.VMEM)],
        out_specs=pl.BlockSpec(memory_space=pl.ANY),
        out_shape=jax.ShapeDtypeStruct(xt.shape, xt.dtype),
        scratch_shapes=[pltpu.VMEM((K, S, W, H), x.dtype),
                        pltpu.VMEM((3, S, 8, 128), jnp.float32),
                        pltpu.SemaphoreType.DMA((NS,)),
                        pltpu.SemaphoreType.DMA((NS,))],
        compiler_params=pltpu.CompilerParams(
            vmem_limit_bytes=120 * 2**20, disable_bounds_checks=True),
    )(xt, g.reshape(C // 128, 128), b.reshape(C // 128, 128))
    return o.reshape(B, C, W, H).transpose(0, 1, 3, 2)
```
